```python
import jax
import jax.numpy as jnp

def _softmax(x, axis=-1):
    return jax.nn.softmax(x, axis=axis)
def _gelu(x):
    return jax.nn.gelu(x, approximate=True)
def _silu(x):
    return jax.nn.silu(x)
def _sigmoid(x):
    return jax.nn.sigmoid(x)
def _layernorm(x, axis=-1, eps=1e-5):
    m = jnp.mean(x, axis=axis, keepdims=True)
    v = jnp.var(x, axis=axis, keepdims=True)
    return (x - m) / jnp.sqrt(v + eps)
def _scatter_add(tgt, idx, src, axis=0):
    return tgt.at[idx].add(src)
def _segment_sum(src, seg, n):
    return jax.ops.segment_sum(src, seg, n)
class _Rng:
    def __init__(self, key):
        self._k = key
    def _next(self):
        self._k, sub = jax.random.split(self._k)
        return sub
    def normal(self, shape):
        return jax.random.normal(self._next(), shape, dtype=jnp.bfloat16)
    def randint(self, lo, hi, shape):
        return jax.random.randint(self._next(), shape, lo, hi, dtype=jnp.int32)
    def uniform(self, shape, lo=0.0, hi=1.0):
        return jax.random.uniform(self._next(), shape, jnp.bfloat16, lo, hi)
    def permutation(self, n):
        return jax.random.permutation(self._next(), n)


kernel_name = 'interleave_layers__linear_kernel_hedgehog__sliding_local_dilated__prompt'

def setup_inputs():
    _rng = _Rng(jax.random.key(int.from_bytes(__import__("os").urandom(4), "little")))
    _w = (lambda a: (lambda t: t.astype(jnp.bfloat16) if jnp.issubdtype(t.dtype, jnp.floating) else t)(jnp.asarray(a)))
    def _A_setup():
        B, S, D, H = 1, 2048, 1024, 32
        Dh = D // H
        return {
            "x": _w((lambda *s: _rng.normal(s) * 0.05)(B, S, D)),
            "wqkv": _w((lambda *s: _rng.normal(s) * 0.05)(D, 3 * D)),
            "w_phi": _w((lambda *s: _rng.normal(s) * 0.05)(H, Dh, Dh) * (Dh ** -0.5)),
            "wo": _w((lambda *s: _rng.normal(s) * 0.05)(D, D)),
        }
    _A_in = _A_setup()

    def _B_setup():
        B, S, D = 1, 2048, 1024
        return {
            "x": _w((lambda *s: _rng.normal(s) * 0.05)(B, S, D)),
            "wqkv": _w((lambda *s: _rng.normal(s) * 0.05)(D, 3 * D)),
            "wo": _w((lambda *s: _rng.normal(s) * 0.05)(D, D)),
        }
    _B_in = _B_setup()

    return {
        "A_x": _A_in["x"],
        "A_wqkv": _A_in["wqkv"],
        "A_w_phi": _A_in["w_phi"],
        "A_wo": _A_in["wo"],
        "B_x": _B_in["x"],
        "B_wqkv": _B_in["wqkv"],
        "B_wo": _B_in["wo"],
    }

def reference(A_x, A_wqkv, A_w_phi, A_wo, B_x, B_wqkv, B_wo):
    def _A_ref(x, wqkv, w_phi, wo):
        B, S, D = x.shape
        H = 32; Dh = D // H
        qkv = (lambda x, *d: x.transpose(*d))((x @ wqkv).reshape(B, S, 3, H, Dh), 2, 0, 3, 1, 4)
        q, k, v = qkv[0], qkv[1], qkv[2]
        pq = jnp.einsum("bhsd,hdf->bhsf", q, w_phi)
        pk = jnp.einsum("bhsd,hdf->bhsf", k, w_phi)
        phi_q = jnp.concatenate([_softmax(pq, axis=-1), _softmax(-pq, axis=-1)], axis=-1)
        phi_k = jnp.concatenate([_softmax(pk, axis=-1), _softmax(-pk, axis=-1)], axis=-1)
        kv = jnp.einsum("bhsf,bhsd->bhfd", phi_k, v)
        z  = jnp.einsum("bhsf->bhf", phi_k)
        num = jnp.einsum("bhqf,bhfd->bhqd", phi_q, kv)
        den = jnp.einsum("bhqf,bhf->bhq", phi_q, z)[..., None] + 1e-6
        o = num / den
        return (lambda x, *d: x.transpose(*d))(o, 0, 2, 1, 3).reshape(B, S, D) @ wo

    def _B_ref(x, wqkv, wo):
        B, S, D = x.shape
        H = 32; Dh = D // H
        W, dil = 8, 2
        qkv = (lambda x, *d: x.transpose(*d))((x @ wqkv).reshape(B, S, 3, H, Dh), 2, 0, 3, 1, 4)
        q, k, v = qkv[0], qkv[1], qkv[2]
        scale = Dh ** -0.5
        pos = jnp.arange(S)
        off = jnp.arange(W) * dil
        idx = pos[:, None] - off[None, :]
        mask = idx >= 0
        idx_c = jnp.where(mask, idx, 0).reshape(-1)
        kg = k[:, :, idx_c, :].reshape(B, H, S, W, Dh)
        vg = v[:, :, idx_c, :].reshape(B, H, S, W, Dh)
        logits = jnp.einsum("bhsd,bhswd->bhsw", q, kg) * scale
        logits = jnp.where(mask[None, None, :, :], logits, -1e9)
        attn = _softmax(logits, axis=-1)
        o = jnp.einsum("bhsw,bhswd->bhsd", attn, vg)
        return (lambda x, *d: x.transpose(*d))(o, 0, 2, 1, 3).reshape(B, S, D) @ wo

    x = A_x
    x = x + _A_ref(_layernorm(x, axis=-1), A_wqkv, A_w_phi, A_wo)
    x = x + _B_ref(_layernorm(x, axis=-1), B_wqkv, B_wo)
    x = x + _A_ref(_layernorm(x, axis=-1), A_wqkv, A_w_phi, A_wo)
    x = x + _B_ref(_layernorm(x, axis=-1), B_wqkv, B_wo)
    return x
```

```python
import functools
import jax
import jax.numpy as jnp
import numpy as np
from jax import lax
from jax.experimental import pallas as pl
from jax.experimental.pallas import tpu as pltpu

bf16 = jnp.bfloat16
f32 = jnp.float32
i32 = jnp.int32

S, D, H, DH = 2048, 1024, 32, 32
T, L = 16, 128
NP = 16
LOG2E = 1.4426950408889634
NT_DIMS = (((1,), (1,)), ((), ()))


def _bf(x):
    return pltpu.bitcast(x, bf16)


def _pk(x):
    return pltpu.bitcast(x, i32)


def _recip(x):
    r = pltpu.reciprocal(x, approx=True)
    return r * (2.0 - x * r)


def _layernorm_T(x):
    x3 = x.reshape(D // 8, 8, L)
    m = jnp.sum(jnp.sum(x3, axis=0), axis=0, keepdims=True) * (1.0 / D)
    xc = x3 - m[None]
    v = jnp.sum(jnp.sum(xc * xc, axis=0), axis=0, keepdims=True) * (1.0 / D)
    r = lax.rsqrt(v + 1e-5)
    return (xc * r[None]).reshape(D, L).astype(bf16)


def _dual_softmax_pair(p):
    p3 = p.reshape(8, 8, L) * LOG2E
    mx = jnp.max(p3, axis=0)
    mx = jnp.maximum(mx, pltpu.roll(mx, 4, 0))
    mx = jnp.maximum(mx, pltpu.roll(mx, 2, 0))
    mn = jnp.min(p3, axis=0)
    mn = jnp.minimum(mn, pltpu.roll(mn, 4, 0))
    mn = jnp.minimum(mn, pltpu.roll(mn, 2, 0))
    ep = jnp.exp2(p3 - mx[None])
    en = jnp.exp2(mn[None] - p3)
    sp = jnp.sum(ep, axis=0)
    sp = sp + pltpu.roll(sp, 4, 0)
    sp = sp + pltpu.roll(sp, 2, 0)
    sn = jnp.sum(en, axis=0)
    sn = sn + pltpu.roll(sn, 4, 0)
    sn = sn + pltpu.roll(sn, 2, 0)
    ep = ep * _recip(sp)[None]
    en = en * _recip(sn)[None]
    return jnp.concatenate([ep.reshape(64, L), en.reshape(64, L)], axis=0).astype(bf16)


def _kernel(x_hbm, wa_hbm, wphi_ref, woa_hbm, wb_hbm, wob_hbm, out_hbm,
            waT, wbT, woaT, wobT, xT, xn, pqk, phiq, phik, vA, oS, numL, sems):
    def ln_to_xn(j):
        xn[j] = _pk(_layernorm_T(xT[j]))

    def qkv_a(j, slot):
        r = jnp.dot(_bf(waT[...]), _bf(xn[j]), preferred_element_type=f32)
        pqk[slot] = r[0:2048]
        v = r[2048:3072].astype(bf16)
        for p in range(NP):
            vA[j, 40 * p:40 * p + 32, :] = _pk(v[64 * p:64 * p + 64])

    def soft_a(j, slot):
        for p in range(NP):
            pq = pqk[slot, 64 * p:64 * p + 64, :]
            phiq[j, 64 * p:64 * p + 64, :] = _pk(_dual_softmax_pair(pq))
            pk = pqk[slot, 1024 + 64 * p:1024 + 64 * p + 64, :]
            phik[j, 64 * p:64 * p + 64, :] = _pk(_dual_softmax_pair(pk))

    def kv_phase():
        r = lax.broadcasted_iota(i32, (80, L), 0)
        c = lax.broadcasted_iota(i32, (80, L), 1)
        hs = jnp.where(r < 64, r // 32, (r - 64) // 8)
        keep = hs == (c % 2)
        for p in range(NP):
            Lm = jnp.concatenate([_bf(vA[j, 40 * p:40 * p + 40, :]) for j in range(T)], axis=1)
            Rm = jnp.concatenate([_bf(phik[j, 64 * p:64 * p + 64, :]) for j in range(T)], axis=1)
            kvT = lax.dot_general(Lm, Rm, NT_DIMS, preferred_element_type=f32)
            numL[p] = _pk(jnp.where(keep, kvT, 0.0).astype(bf16))

    def num_phase():
        for p in range(NP):
            Rm = jnp.concatenate([_bf(phiq[j, 64 * p:64 * p + 64, :]) for j in range(T)], axis=1)
            nd = jnp.dot(_bf(numL[p]), Rm, preferred_element_type=f32)
            for j in range(T):
                t = nd[:, L * j:L * (j + 1)]
                r0 = _recip(t[64:72] + 1e-6)
                r1 = _recip(t[72:80] + 1e-6)
                o0 = (t[0:32].reshape(4, 8, L) * r0[None]).reshape(32, L)
                o1 = (t[32:64].reshape(4, 8, L) * r1[None]).reshape(32, L)
                oS[j, 32 * p:32 * p + 32, :] = _pk(jnp.concatenate([o0, o1], axis=0).astype(bf16))

    def oproj(j, woT):
        y = jnp.dot(_bf(woT[...]), _bf(oS[j]), preferred_element_type=f32)
        xT[j] = xT[j] + y

    def qkv_b(j, qB, kext, vext):
        r = jnp.dot(_bf(wbT[...]), _bf(xn[j]), preferred_element_type=f32)
        qB[j] = r[0:1024]
        k = r[1024:2048]
        v = r[2048:3072]
        kext[j + 14] = k
        vext[j + 14] = v
        rs = jnp.where(j >= 2, j - 2, j + 30) if not isinstance(j, int) else (j - 2 if j >= 2 else j + 30)
        kext[rs] = pltpu.roll(k, 1, 1)
        vext[rs] = pltpu.roll(v, 1, 1)

    lane_ok = lax.broadcasted_iota(i32, (8, L), 1) >= 1

    def attn_b(j, qB, kext, vext):
        scale = DH ** -0.5 * LOG2E
        for h in range(H):
            rows = slice(h * 32, (h + 1) * 32)
            q = qB[j, rows, :].reshape(4, 8, L)
            logits = []
            for w in range(8):
                k = kext[j + 14 - 2 * w, rows, :].reshape(4, 8, L)
                s = jnp.sum(q * k, axis=0)
                s = s + pltpu.roll(s, 4, 0)
                s = s + pltpu.roll(s, 2, 0)
                s = s + pltpu.roll(s, 1, 0)
                if w > 0:
                    s = jnp.where(jnp.logical_or(lane_ok, j >= 2 * w), s, -1e9)
                logits.append(s)
            m = logits[0]
            for w in range(1, 8):
                m = jnp.maximum(m, logits[w])
            es = [jnp.exp2((l - m) * scale) for l in logits]
            ssum = es[0]
            for w in range(1, 8):
                ssum = ssum + es[w]
            r = _recip(ssum)
            acc = None
            for w in range(8):
                v = vext[j + 14 - 2 * w, rows, :].reshape(4, 8, L)
                t = v * (es[w] * r)[None]
                acc = t if acc is None else acc + t
            oS[j, 16 * h:16 * h + 16, :] = _pk(acc.reshape(32, L).astype(bf16))

    def scope1(xraw, waraw, woaraw, wbraw, wobraw):
        def cp(i):
            if i < 8:
                return pltpu.make_async_copy(x_hbm.at[:, pl.ds(i * L, L)], xraw.at[i], sems.at[i])
            i2 = i - 8
            if i2 < 24:
                return pltpu.make_async_copy(wa_hbm.at[:, pl.ds(i2 * L, L)], waraw.at[i2], sems.at[i])
            i2 -= 24
            if i2 < 24:
                return pltpu.make_async_copy(wb_hbm.at[:, pl.ds(i2 * L, L)], wbraw.at[i2], sems.at[i])
            i2 -= 24
            if i2 < 8:
                return pltpu.make_async_copy(woa_hbm.at[:, pl.ds(i2 * L, L)], woaraw.at[i2], sems.at[i])
            i2 -= 8
            return pltpu.make_async_copy(wob_hbm.at[:, pl.ds(i2 * L, L)], wobraw.at[i2], sems.at[i])
        for i in range(72):
            cp(i).start()

        ones = jnp.full((8, L), 0x3F803F80, i32)
        for j in range(T):
            for p in range(NP):
                vA[j, 40 * p + 32:40 * p + 40, :] = ones

        xv = xraw.bitcast(i32)
        for c in range(8):
            cp(c).wait()
            for jj in range(8):
                wt = xv[c, pl.ds(jj, L, stride=8), :].T
                xT[2 * jj, c * L:(c + 1) * L, :] = pltpu.bitcast(wt << 16, f32)
                xT[2 * jj + 1, c * L:(c + 1) * L, :] = pltpu.bitcast(wt & jnp.int32(-65536), f32)
        ln_to_xn(0)

        rr = lax.broadcasted_iota(i32, (L, L), 0)
        cc = lax.broadcasted_iota(i32, (L, L), 1)
        h_out = (rr // 64) * 2 + (rr % 2)
        keep = h_out == (cc // 32)
        re = lax.broadcasted_iota(i32, (L, DH), 0)
        ce = lax.broadcasted_iota(i32, (L, DH), 1)
        f_out = ((re % 64) // 8) * 4 + (re % 8) // 2
        E = jnp.where(f_out == ce, 1.0, 0.0).astype(bf16)
        G = []
        for c in range(8):
            g = lax.dot_general(E, wphi_ref[c * L:(c + 1) * L, :], NT_DIMS, preferred_element_type=f32)
            G.append(jnp.where(keep, g, 0.0).astype(bf16))
        for c in range(16):
            cp(8 + c).wait()
            wt = lax.dot_general(G[c % 8], waraw[c], NT_DIMS, preferred_element_type=f32)
            waT[64 * c:64 * c + 64, :] = _pk(wt.astype(bf16))
        for c in range(16, 24):
            cp(8 + c).wait()
            waT[64 * c:64 * c + 64, :] = _pk(waraw[c].T)

        def xpose_b(c):
            wbT[pl.ds(pl.multiple_of(64 * c, 64), 64), :] = _pk(wbraw[c].T)

        qkv_a(0, 0)
        ln_to_xn(1)

        def body(i, carry):
            soft_a(i - 1, (i - 1) % 2)
            qkv_a(i, i % 2)
            ln_to_xn(jnp.minimum(i + 1, T - 1))
            return carry
        lax.fori_loop(1, T, body, 0)
        soft_a(T - 1, (T - 1) % 2)

        for c in range(24):
            cp(32 + c).wait()
            wbT[64 * c:64 * c + 64, :] = _pk(wbraw[c].T)
        for c in range(8):
            cp(56 + c).wait()
            woaT[64 * c:64 * c + 64, :] = _pk(woaraw[c].T)
        for c in range(8):
            cp(64 + c).wait()
            wobT[64 * c:64 * c + 64, :] = _pk(wobraw[c].T)

    pl.run_scoped(scope1,
                  pltpu.VMEM((8, S, L), bf16), pltpu.VMEM((24, D, L), bf16), pltpu.VMEM((8, D, L), bf16),
                  pltpu.VMEM((24, D, L), bf16), pltpu.VMEM((8, D, L), bf16))

    def scope2(qB, kext, vext, ostage):
        def b1_loop():
            oproj(0, woaT)
            ln_to_xn(0)

            def body(i, carry):
                oproj(i + 1, woaT)
                qkv_b(i, qB, kext, vext)
                ln_to_xn(i + 1)
                return carry
            lax.fori_loop(0, T - 1, body, 0)
            qkv_b(T - 1, qB, kext, vext)

        kv_phase()
        num_phase()
        b1_loop()

        attn_b(0, qB, kext, vext)
        oproj(0, wobT)
        attn_b(1, qB, kext, vext)
        ln_to_xn(0)
        oproj(1, wobT)
        qkv_a(0, 0)
        attn_b(2, qB, kext, vext)
        ln_to_xn(1)

        def body2(i, carry):
            oproj(i, wobT)
            soft_a(i - 2, i % 2)
            qkv_a(i - 1, (i - 1) % 2)
            attn_b(i + 1, qB, kext, vext)
            ln_to_xn(i)
            return carry
        lax.fori_loop(2, T - 1, body2, 0)
        oproj(T - 1, wobT)
        soft_a(T - 3, (T - 3) % 2)
        qkv_a(T - 2, (T - 2) % 2)
        ln_to_xn(T - 1)
        soft_a(T - 2, (T - 2) % 2)
        qkv_a(T - 1, (T - 1) % 2)
        soft_a(T - 1, (T - 1) % 2)

        kv_phase()
        num_phase()
        b1_loop()

        attn_b(0, qB, kext, vext)

        def body3(i, carry):
            oproj(i, wobT)
            attn_b(i + 1, qB, kext, vext)
            return carry
        lax.fori_loop(0, T - 1, body3, 0)
        oproj(T - 1, wobT)

        ov = ostage.bitcast(i32)

        def rne(u):
            return u + 0x7FFF + ((u >> 16) & 1)
        for c in range(8):
            for jj in range(8):
                a = pltpu.bitcast(xT[2 * jj, c * L:(c + 1) * L, :], i32)
                b = pltpu.bitcast(xT[2 * jj + 1, c * L:(c + 1) * L, :], i32)
                wv = lax.shift_right_logical(rne(a), 16) | (rne(b) & jnp.int32(-65536))
                ov[c, pl.ds(jj, L, stride=8), :] = wv.T
            pltpu.make_async_copy(ostage.at[c], out_hbm.at[:, pl.ds(c * L, L)], sems.at[c]).start()
        for c in range(8):
            pltpu.make_async_copy(ostage.at[c], out_hbm.at[:, pl.ds(c * L, L)], sems.at[c]).wait()

    pl.run_scoped(scope2,
                  pltpu.VMEM((T, D, L), f32), pltpu.VMEM((32, D, L), f32), pltpu.VMEM((32, D, L), f32),
                  pltpu.VMEM((8, S, L), bf16))


@jax.jit
def pallas_interleave_layers__linear_kernel_hedgehog__sliding_local_dilated__prompt_kernel(
        A_x, A_wqkv, A_w_phi, A_wo, B_x, B_wqkv, B_wo):
    del B_x
    x = A_x.reshape(S, D)
    wphi = A_w_phi.reshape(H * DH, DH)
    any_spec = pl.BlockSpec(memory_space=pl.ANY)
    out = pl.pallas_call(
        _kernel,
        out_shape=jax.ShapeDtypeStruct((S, D), bf16),
        in_specs=[any_spec, any_spec, pl.BlockSpec(memory_space=pltpu.VMEM), any_spec, any_spec, any_spec],
        out_specs=any_spec,
        scratch_shapes=[
            pltpu.VMEM((1536, D), i32),
            pltpu.VMEM((1536, D), i32),
            pltpu.VMEM((512, D), i32),
            pltpu.VMEM((512, D), i32),
            pltpu.VMEM((T, D, L), f32),
            pltpu.VMEM((T, 512, L), i32),
            pltpu.VMEM((2, 2048, L), f32),
            pltpu.VMEM((T, 1024, L), i32),
            pltpu.VMEM((T, 1024, L), i32),
            pltpu.VMEM((T, 640, L), i32),
            pltpu.VMEM((T, 512, L), i32),
            pltpu.VMEM((NP, 40, L), i32),
            pltpu.SemaphoreType.DMA((72,)),
        ],
        compiler_params=pltpu.CompilerParams(vmem_limit_bytes=120 * 1024 * 1024),
        name="hedgehog_fused",
    )(x, A_wqkv, wphi, A_wo, B_wqkv, B_wo)
    return out.reshape(1, S, D)
```

```python
import jax
import jax.numpy as jnp
from jax import lax
from jax.experimental import pallas as pl
from jax.experimental.pallas import tpu as pltpu

bf16 = jnp.bfloat16
f32 = jnp.float32
i32 = jnp.int32

S, D, H, DH = 2048, 1024, 32, 32
T, L = 16, 128
NP = 16
LOG2E = 1.4426950408889634
NT_DIMS = (((1,), (1,)), ((), ()))


def _bf(x):
    return pltpu.bitcast(x, bf16)


def _pk(x):
    return pltpu.bitcast(x, i32)


def _recip(x):
    r = pltpu.reciprocal(x, approx=True)
    return r * (2.0 - x * r)


def _layernorm(xT, j, store):
    CH = 64
    n = D // CH
    acc = [None] * 4
    for c in range(n):
        s = jnp.sum(xT[j, c * CH:(c + 1) * CH, :].reshape(CH // 8, 8, L), axis=0)
        acc[c % 4] = s if acc[c % 4] is None else acc[c % 4] + s
    m = jnp.sum((acc[0] + acc[1]) + (acc[2] + acc[3]), axis=0, keepdims=True) * (1.0 / D)
    mb = jnp.broadcast_to(m, (8, L))
    acc = [None] * 4
    CH2 = CH // 2
    for c in range(2 * n):
        x = xT[j, c * CH2:(c + 1) * CH2, :].reshape(CH2 // 8, 8, L) - mb[None]
        s = jnp.sum(x * x, axis=0)
        acc[c % 4] = s if acc[c % 4] is None else acc[c % 4] + s
    v = jnp.sum((acc[0] + acc[1]) + (acc[2] + acc[3]), axis=0, keepdims=True) * (1.0 / D)
    r = jnp.broadcast_to(lax.rsqrt(v + 1e-5), (8, L))
    CH3 = CH // 4
    for c in range(4 * n):
        x = (xT[j, c * CH3:(c + 1) * CH3, :].reshape(CH3 // 8, 8, L) - mb[None]) * r[None]
        store(c * CH3, CH3, x.reshape(CH3, L).astype(bf16))


def _dual_softmax_pair(p):
    p3 = p.reshape(8, 8, L) * LOG2E
    mx = jnp.max(p3, axis=0)
    mx = jnp.maximum(mx, pltpu.roll(mx, 4, 0))
    mx = jnp.maximum(mx, pltpu.roll(mx, 2, 0))
    mn = jnp.min(p3, axis=0)
    mn = jnp.minimum(mn, pltpu.roll(mn, 4, 0))
    mn = jnp.minimum(mn, pltpu.roll(mn, 2, 0))
    ep = jnp.exp2(p3 - mx[None])
    en = jnp.exp2(mn[None] - p3)
    sp = jnp.sum(ep, axis=0)
    sp = sp + pltpu.roll(sp, 4, 0)
    sp = sp + pltpu.roll(sp, 2, 0)
    sn = jnp.sum(en, axis=0)
    sn = sn + pltpu.roll(sn, 4, 0)
    sn = sn + pltpu.roll(sn, 2, 0)
    ep = ep * _recip(sp)[None]
    en = en * _recip(sn)[None]
    return jnp.concatenate([ep.reshape(64, L), en.reshape(64, L)], axis=0).astype(bf16)


def _tie(x, dep, zero):
    return pltpu.bitcast(pltpu.bitcast(x, i32) | (pltpu.bitcast(dep, i32) & zero), f32)


def _kernel(x_hbm, wa_hbm, wphi_ref, woa_hbm, wb_hbm, wob_hbm, out_hbm,
            waT, wbT, woaT, wobT, wobraw, xT, xn, xnE, xnO, pqkE, pqkO, phiq, phik, vA, oS, numL, sems):
    zero = lax.broadcasted_iota(i32, (8, L), 1) >> 10
    lane_ok = lax.broadcasted_iota(i32, (8, L), 1) >= 1

    def ln(j, dst):
        def store(r0, n, val):
            dst[r0:r0 + n, :] = val
        _layernorm(xT, j, store)

    def ln_arr(j):
        def store(r0, n, val):
            xn[j, r0:r0 + n, :] = val
        _layernorm(xT, j, store)

    def qkv_a(j, src, pqk):
        r = jnp.dot(_bf(waT[...]), src[...], preferred_element_type=f32)
        pqk[...] = r[0:2048]
        v = r[2048:3072].astype(bf16)
        for p in range(NP):
            vA[j, 80 * p:80 * p + 64, :] = v[64 * p:64 * p + 64]

    def soft_a(j, pqk):
        for p in range(NP):
            phiq[j, 128 * p:128 * p + 128, :] = _dual_softmax_pair(pqk[64 * p:64 * p + 64, :])
            phik[j, 128 * p:128 * p + 128, :] = _dual_softmax_pair(pqk[1024 + 64 * p:1024 + 64 * p + 64, :])

    def kv_phase():
        r = lax.broadcasted_iota(i32, (80, L), 0)
        c = lax.broadcasted_iota(i32, (80, L), 1)
        hs = jnp.where(r < 64, r // 32, (r - 64) // 8)
        keep = hs == (c % 2)
        for p in range(NP):
            Lm = jnp.concatenate([vA[j, 80 * p:80 * p + 80, :] for j in range(T)], axis=1)
            Rm = jnp.concatenate([phik[j, 128 * p:128 * p + 128, :] for j in range(T)], axis=1)
            kvT = lax.dot_general(Lm, Rm, NT_DIMS, preferred_element_type=f32)
            numL[p] = jnp.where(keep, kvT, 0.0).astype(bf16)

    def num_phase():
        for p in range(NP):
            Rm = jnp.concatenate([phiq[j, 128 * p:128 * p + 128, :] for j in range(T)], axis=1)
            nd = jnp.dot(numL[p], Rm, preferred_element_type=f32)
            for j in range(T):
                t = nd[:, L * j:L * (j + 1)]
                r0 = _recip(t[64:72] + 1e-6)
                r1 = _recip(t[72:80] + 1e-6)
                o0 = (t[0:32].reshape(4, 8, L) * r0[None]).reshape(32, L)
                o1 = (t[32:64].reshape(4, 8, L) * r1[None]).reshape(32, L)
                oS[j, 64 * p:64 * p + 64, :] = jnp.concatenate([o0, o1], axis=0).astype(bf16)

    def oproj(j, woT):
        y = jnp.dot(_bf(woT[...]), oS[j], preferred_element_type=f32)
        xT[j] = xT[j] + y

    def qkv_b(j, m, q_ref, k_ref, v_ref):
        r = jnp.dot(_bf(wbT[...]), xn[j], preferred_element_type=f32)
        CH = 64
        for ref, off in ((k_ref, 0), (v_ref, 1024)):
            for c in range(D // CH):
                val = r[off + c * CH:off + (c + 1) * CH]
                ref[m + 8, c * CH:(c + 1) * CH, :] = val
                ref[m, c * CH:(c + 1) * CH, :] = pltpu.roll(val, 1, 1)
        q_ref[m] = r[2048:3072]

    def attn_b(j, m, q_ref, k_ref, v_ref, chain):
        scale = DH ** -0.5 * LOG2E
        dep = None
        for h in range(H):
            rows = slice(h * 32, (h + 1) * 32)
            q = q_ref[m, rows, :].reshape(4, 8, L)
            qs = [q[i] for i in range(4)]
            if chain and dep is not None:
                qs[0] = _tie(qs[0], dep, zero)
            logits = []
            for w in range(8):
                k = k_ref[m + 8 - w, rows, :].reshape(4, 8, L)
                s = (qs[0] * k[0] + qs[1] * k[1]) + (qs[2] * k[2] + qs[3] * k[3])
                s = s + pltpu.roll(s, 4, 0)
                s = s + pltpu.roll(s, 2, 0)
                s = s + pltpu.roll(s, 1, 0)
                if w > 0 and not (isinstance(m, int) and m >= w):
                    s = jnp.where(jnp.logical_or(lane_ok, m >= w), s, -1e9)
                logits.append(s)
            mx = logits[0]
            for w in range(1, 8):
                mx = jnp.maximum(mx, logits[w])
            es = [jnp.exp2((l - mx) * scale) for l in logits]
            ssum = es[0]
            for w in range(1, 8):
                ssum = ssum + es[w]
            r = _recip(ssum)
            acc = None
            for w in range(8):
                v = v_ref[m + 8 - w, rows, :].reshape(4, 8, L)
                t = v * es[w][None]
                acc = t if acc is None else acc + t
            o = acc * r[None]
            dep = o[0]
            oS[j, rows, :] = o.reshape(32, L).astype(bf16)

    def cp_wob(c):
        return pltpu.make_async_copy(wob_hbm.at[:, pl.ds(c * L, L)], wobraw.at[c], sems.at[64 + c])

    def scope1(xraw, waraw, woaraw, wbraw):
        def cp(i):
            if i < 8:
                return pltpu.make_async_copy(x_hbm.at[:, pl.ds(i * L, L)], xraw.at[i], sems.at[i])
            i2 = i - 8
            if i2 < 24:
                return pltpu.make_async_copy(wa_hbm.at[:, pl.ds(i2 * L, L)], waraw.at[i2], sems.at[i])
            i2 -= 24
            if i2 < 24:
                src = (i2 + 8) % 24
                return pltpu.make_async_copy(wb_hbm.at[:, pl.ds(src * L, L)], wbraw.at[i2], sems.at[i])
            i2 -= 24
            return pltpu.make_async_copy(woa_hbm.at[:, pl.ds(i2 * L, L)], woaraw.at[i2], sems.at[i])
        for i in range(64):
            cp(i).start()
        for c in range(8):
            cp_wob(c).start()

        ones = jnp.ones((16, L), bf16)
        for j in range(T):
            for p in range(NP):
                vA[j, 80 * p + 64:80 * p + 80, :] = ones

        xv = xraw.bitcast(i32)
        for c in range(8):
            cp(c).wait()
            for jj in range(8):
                wt = xv[c, pl.ds(jj, L, stride=8), :].T
                xT[jj, c * L:(c + 1) * L, :] = pltpu.bitcast(wt << 16, f32)
                xT[8 + jj, c * L:(c + 1) * L, :] = pltpu.bitcast(wt & jnp.int32(-65536), f32)
        ln(0, xnE)
        ln(8, xnO)

        rr = lax.broadcasted_iota(i32, (L, L), 0)
        cc = lax.broadcasted_iota(i32, (L, L), 1)
        h_out = (rr // 64) * 2 + (rr % 2)
        keep = h_out == (cc // 32)
        re = lax.broadcasted_iota(i32, (L, DH), 0)
        ce = lax.broadcasted_iota(i32, (L, DH), 1)
        f_out = ((re % 64) // 8) * 4 + (re % 8) // 2
        E = jnp.where(f_out == ce, 1.0, 0.0).astype(bf16)
        G = []
        for c in range(8):
            g = lax.dot_general(E, wphi_ref[c * L:(c + 1) * L, :], NT_DIMS, preferred_element_type=f32)
            G.append(jnp.where(keep, g, 0.0).astype(bf16))
        for c in range(16):
            cp(8 + c).wait()
            wt = lax.dot_general(G[c % 8], waraw[c], NT_DIMS, preferred_element_type=f32)
            waT[64 * c:64 * c + 64, :] = _pk(wt.astype(bf16))
        for c in range(16, 24):
            cp(8 + c).wait()
            waT[64 * c:64 * c + 64, :] = _pk(waraw[c].T)

        def wait_wb(c):
            pltpu.make_async_copy(wb_hbm.at[:, pl.ds(0, L)], wbraw.at[c], sems.at[32 + c]).wait()

        def xpose_wb(c):
            wbT[pl.ds(pl.multiple_of(64 * c, 64), 64), :] = _pk(wbraw[c].T)

        qkv_a(0, xnE, pqkE)
        qkv_a(8, xnO, pqkO)
        ln(1, xnE)
        ln(9, xnO)

        def body(t, carry, nblk=4):
            for u in range(nblk):
                wait_wb(4 * (t - 1) + u)
            soft_a(t - 1, pqkE)
            soft_a(t + 7, pqkO)
            qkv_a(t, xnE, pqkE)
            qkv_a(t + 8, xnO, pqkO)
            ln(t + 1, xnE)
            ln(t + 9, xnO)
            for u in range(nblk):
                xpose_wb(4 * (t - 1) + u)
            return carry
        lax.fori_loop(1, 7, body, 0)
        for c in range(8):
            cp(56 + c).wait()
        soft_a(6, pqkE)
        soft_a(14, pqkO)
        qkv_a(7, xnE, pqkE)
        qkv_a(15, xnO, pqkO)
        for c in range(8):
            woaT[64 * c:64 * c + 64, :] = _pk(woaraw[c].T)
        soft_a(7, pqkE)
        soft_a(15, pqkO)
        kv_phase()

    pl.run_scoped(scope1,
                  pltpu.VMEM((8, S, L), bf16), pltpu.VMEM((24, D, L), bf16), pltpu.VMEM((8, D, L), bf16),
                  pltpu.VMEM((24, D, L), bf16))

    def scope2(qE, kE, vE, qO, kO, vO, ostage):
        def attn_e(m, chain=True):
            attn_b(m, m, qE, kE, vE, chain)

        def attn_o(m, chain=True):
            attn_b(m + 8, m, qO, kO, vO, chain)

        def b1(first):
            num_phase()
            oproj(0, woaT)
            oproj(1, woaT)
            ln_arr(0)

            def bodyx(i, carry):
                if first:
                    cp_wob(i).wait()
                oproj(i + 2, woaT)
                qkv_b(i, i, qE, kE, vE)
                ln_arr(i + 1)
                if first:
                    wobT[pl.ds(pl.multiple_of(64 * i, 64), 64), :] = _pk(wobraw[i].T)
                return carry
            lax.fori_loop(0, 8, bodyx, 0)

            def bodyy(i, carry, do_o=True, do_ln=True):
                if do_o:
                    oproj(i + 2, woaT)
                attn_e(i - 8)
                qkv_b(i, i - 8, qO, kO, vO)
                if do_ln:
                    ln_arr(i + 1)
                return carry
            lax.fori_loop(8, 14, bodyy, 0)
            bodyy(14, 0, do_o=False)
            bodyy(15, 0, do_o=False, do_ln=False)

        b1(True)
        oproj(0, wobT)
        attn_o(0, False)
        oproj(8, wobT)
        attn_o(1, False)
        oproj(1, wobT)
        oproj(9, wobT)
        ln(0, xnE)
        ln(8, xnO)
        attn_o(2, False)

        def bodyz(t, carry):
            oproj(t + 1, wobT)
            oproj(t + 9, wobT)
            soft_a(jnp.maximum(t - 2, 0), pqkE)
            soft_a(jnp.maximum(t - 2, 0) + 8, pqkO)
            qkv_a(t - 1, xnE, pqkE)
            qkv_a(t + 7, xnO, pqkO)
            ln(t, xnE)
            ln(t + 8, xnO)
            attn_o(jnp.minimum(t + 2, 7))
            return carry
        lax.fori_loop(1, 7, bodyz, 0)
        soft_a(5, pqkE)
        soft_a(13, pqkO)
        qkv_a(6, xnE, pqkE)
        qkv_a(14, xnO, pqkO)
        ln(7, xnE)
        ln(15, xnO)
        soft_a(6, pqkE)
        soft_a(14, pqkO)
        qkv_a(7, xnE, pqkE)
        qkv_a(15, xnO, pqkO)
        soft_a(7, pqkE)
        soft_a(15, pqkO)
        kv_phase()

        b1(False)
        ov = ostage.bitcast(i32)
        out3 = out_hbm.reshape(L, 16, D)

        def rne(u):
            return u + 0x7FFF + ((u >> 16) & 1)

        def pack(t):
            for c in range(8):
                a = pltpu.bitcast(xT[t, c * L:(c + 1) * L, :], i32)
                b = pltpu.bitcast(xT[t + 8, c * L:(c + 1) * L, :], i32)
                wv = lax.shift_right_logical(rne(a), 16) | (rne(b) & jnp.int32(-65536))
                ov[c, :, t, :] = wv.T

        def out_cp(hf, c):
            return pltpu.make_async_copy(ostage.at[c, :, pl.ds(8 * hf, 8), :],
                                         out3.at[:, pl.ds(8 * hf, 8), pl.ds(c * L, L)], sems.at[8 * hf + c])

        oproj(0, wobT)
        oproj(1, wobT)
        attn_o(0, False)

        def bodyf(t, carry):
            oproj(t + 2, wobT)
            oproj(t + 8, wobT)
            attn_o(t + 1)
            pack(jnp.maximum(t - 1, 0))
            return carry
        lax.fori_loop(0, 5, bodyf, 0)
        for c in range(8):
            out_cp(0, c).start()
        bodyf(5, 0)
        oproj(14, wobT)
        attn_o(7, False)
        pack(5)
        oproj(15, wobT)
        pack(6)
        pack(7)
        for c in range(8):
            out_cp(1, c).start()
        for hf in range(2):
            for c in range(8):
                out_cp(hf, c).wait()

    pl.run_scoped(scope2,
                  pltpu.VMEM((8, D, L), f32), pltpu.VMEM((16, D, L), f32), pltpu.VMEM((16, D, L), f32),
                  pltpu.VMEM((8, D, L), f32), pltpu.VMEM((16, D, L), f32), pltpu.VMEM((16, D, L), f32),
                  pltpu.VMEM((8, L, 16, L), bf16))


@jax.jit
def pallas_interleave_layers__linear_kernel_hedgehog__sliding_local_dilated__prompt_kernel(
        A_x, A_wqkv, A_w_phi, A_wo, B_x, B_wqkv, B_wo):
    del B_x
    x = A_x.reshape(S, D)
    wphi = A_w_phi.reshape(H * DH, DH)
    any_spec = pl.BlockSpec(memory_space=pl.ANY)
    out = pl.pallas_call(
        _kernel,
        out_shape=jax.ShapeDtypeStruct((S, D), bf16),
        in_specs=[any_spec, any_spec, pl.BlockSpec(memory_space=pltpu.VMEM), any_spec, any_spec, any_spec],
        out_specs=any_spec,
        scratch_shapes=[
            pltpu.VMEM((1536, D), i32),
            pltpu.VMEM((1536, D), i32),
            pltpu.VMEM((512, D), i32),
            pltpu.VMEM((512, D), i32),
            pltpu.VMEM((8, D, L), bf16),
            pltpu.VMEM((T, D, L), f32),
            pltpu.VMEM((T, D, L), bf16),
            pltpu.VMEM((D, L), bf16),
            pltpu.VMEM((D, L), bf16),
            pltpu.VMEM((2048, L), f32),
            pltpu.VMEM((2048, L), f32),
            pltpu.VMEM((T, 2048, L), bf16),
            pltpu.VMEM((T, 2048, L), bf16),
            pltpu.VMEM((T, 1280, L), bf16),
            pltpu.VMEM((T, D, L), bf16),
            pltpu.VMEM((NP, 80, L), bf16),
            pltpu.SemaphoreType.DMA((72,)),
        ],
        compiler_params=pltpu.CompilerParams(vmem_limit_bytes=120 * 1024 * 1024),
        name="hedgehog_fused",
    )(x, A_wqkv, wphi, A_wo, B_wqkv, B_wo)
    return out.reshape(1, S, D)
```

```python
import jax
import jax.numpy as jnp
import numpy as np
from jax import lax
from jax.experimental import pallas as pl
from jax.experimental.pallas import tpu as pltpu

bf16 = jnp.bfloat16
f32 = jnp.float32
i32 = jnp.int32

S, D, H, DH = 2048, 1024, 32, 32
T, L = 16, 128
NP = 16
LOG2E = 1.4426950408889634
NT_DIMS = (((1,), (1,)), ((), ()))


def _bf(x):
    return pltpu.bitcast(x, bf16)


def _pk(x):
    return pltpu.bitcast(x, i32)


def _recip(x):
    r = pltpu.reciprocal(x, approx=True)
    return r * (2.0 - x * r)


def _layernorm(xT, j, store):
    CH = 64
    n = D // CH
    acc = [None] * 4
    for c in range(n):
        s = jnp.sum(xT[j, c * CH:(c + 1) * CH, :].reshape(CH // 8, 8, L), axis=0)
        acc[c % 4] = s if acc[c % 4] is None else acc[c % 4] + s
    m = jnp.sum((acc[0] + acc[1]) + (acc[2] + acc[3]), axis=0, keepdims=True) * (1.0 / D)
    mb = jnp.broadcast_to(m, (8, L))
    acc = [None] * 4
    CH2 = CH // 2
    for c in range(2 * n):
        x = xT[j, c * CH2:(c + 1) * CH2, :].reshape(CH2 // 8, 8, L) - mb[None]
        s = jnp.sum(x * x, axis=0)
        acc[c % 4] = s if acc[c % 4] is None else acc[c % 4] + s
    v = jnp.sum((acc[0] + acc[1]) + (acc[2] + acc[3]), axis=0, keepdims=True) * (1.0 / D)
    r = jnp.broadcast_to(lax.rsqrt(v + 1e-5), (8, L))
    CH3 = CH // 4
    for c in range(4 * n):
        x = (xT[j, c * CH3:(c + 1) * CH3, :].reshape(CH3 // 8, 8, L) - mb[None]) * r[None]
        store(c * CH3, CH3, x.reshape(CH3, L).astype(bf16))


def _dual_softmax_pair(p):
    p3 = p.reshape(8, 8, L) * LOG2E
    mx = jnp.max(p3, axis=0)
    mx = jnp.maximum(mx, pltpu.roll(mx, 4, 0))
    mx = jnp.maximum(mx, pltpu.roll(mx, 2, 0))
    mn = jnp.min(p3, axis=0)
    mn = jnp.minimum(mn, pltpu.roll(mn, 4, 0))
    mn = jnp.minimum(mn, pltpu.roll(mn, 2, 0))
    ep = jnp.exp2(p3 - mx[None])
    en = jnp.exp2(mn[None] - p3)
    sp = jnp.sum(ep, axis=0)
    sp = sp + pltpu.roll(sp, 4, 0)
    sp = sp + pltpu.roll(sp, 2, 0)
    sn = jnp.sum(en, axis=0)
    sn = sn + pltpu.roll(sn, 4, 0)
    sn = sn + pltpu.roll(sn, 2, 0)
    ep = ep * _recip(sp)[None]
    en = en * _recip(sn)[None]
    return jnp.concatenate([ep.reshape(64, L), en.reshape(64, L)], axis=0).astype(bf16)


def _tie(x, dep, zero):
    return pltpu.bitcast(pltpu.bitcast(x, i32) | (pltpu.bitcast(dep, i32) & zero), f32)


def _kernel(one_ref, x_hbm, wa_hbm, wphi_ref, woa_hbm, wb_hbm, wob_hbm, out_hbm,
            waT, wbT, woaT, wobT, wobraw, xT, xn, xnE, xnO, pqkE, pqkO, phiq, phik, vA, oS, oB, numL, sems):
    def region(fn, *args):
        def run():
            fn(*args)
        pl.when(one_ref[0] > 0)(run)

    zero = lax.broadcasted_iota(i32, (8, L), 1) >> 10
    lane_ok = lax.broadcasted_iota(i32, (8, L), 1) >= 1

    def ln(j, dst):
        def store(r0, n, val):
            dst[r0:r0 + n, :] = val
        _layernorm(xT, j, store)

    def xn_tmp(j):
        return xn.at[j]

    def ln_arr(j):
        def store(r0, n, val):
            xn[j, r0:r0 + n, :] = val
        _layernorm(xT, j, store)

    def qkv_a(j, src, pqk):
        r = jnp.dot(_bf(waT[...]), src[...], preferred_element_type=f32)
        pqk[...] = r[0:2048]
        v = r[2048:3072].astype(bf16)
        for p in range(NP):
            vA[j, 80 * p:80 * p + 64, :] = v[64 * p:64 * p + 64]

    def soft_a(j, pqk):
        for p in range(NP):
            phiq[j, 128 * p:128 * p + 128, :] = _dual_softmax_pair(pqk[64 * p:64 * p + 64, :])
            phik[j, 128 * p:128 * p + 128, :] = _dual_softmax_pair(pqk[1024 + 64 * p:1024 + 64 * p + 64, :])

    def kv_phase():
        r = lax.broadcasted_iota(i32, (80, L), 0)
        c = lax.broadcasted_iota(i32, (80, L), 1)
        hs = jnp.where(r < 64, r // 32, (r - 64) // 8)
        keep = hs == (c % 2)
        for p in range(NP):
            Lm = jnp.concatenate([vA[j, 80 * p:80 * p + 80, :] for j in range(T)], axis=1)
            Rm = jnp.concatenate([phik[j, 128 * p:128 * p + 128, :] for j in range(T)], axis=1)
            kvT = lax.dot_general(Lm, Rm, NT_DIMS, preferred_element_type=f32)
            numL[p] = jnp.where(keep, kvT, 0.0).astype(bf16)

    def num_phase():
        for p in range(NP):
            Rm = jnp.concatenate([phiq[j, 128 * p:128 * p + 128, :] for j in range(T)], axis=1)
            nd = jnp.dot(numL[p], Rm, preferred_element_type=f32)
            for j in range(T):
                t = nd[:, L * j:L * (j + 1)]
                r0 = _recip(t[64:72] + 1e-6)
                r1 = _recip(t[72:80] + 1e-6)
                o0 = (t[0:32].reshape(4, 8, L) * r0[None]).reshape(32, L)
                o1 = (t[32:64].reshape(4, 8, L) * r1[None]).reshape(32, L)
                oS[j, 64 * p:64 * p + 64, :] = jnp.concatenate([o0, o1], axis=0).astype(bf16)

    def oproj(j, woT, odd_b=False):
        src = oB[j - 8] if odd_b else oS[j]
        y = jnp.dot(_bf(woT[...]), src, preferred_element_type=f32)
        xT[j] = xT[j] + y

    def qkv_b(j, m, q_ref, k_ref, v_ref):
        r = jnp.dot(_bf(wbT[...]), xn[j], preferred_element_type=f32)
        CH = 64
        for ref, off in ((k_ref, 0), (v_ref, 1024)):
            for c in range(D // CH):
                val = r[off + c * CH:off + (c + 1) * CH]
                ref[m + 8, c * CH:(c + 1) * CH, :] = val
                ref[m, c * CH:(c + 1) * CH, :] = pltpu.roll(val, 1, 1)
        q_ref[m] = r[2048:3072]

    def attn_b(dst, m, q_ref, k_ref, v_ref, chain):
        scale = DH ** -0.5 * LOG2E
        dep = None
        for h in range(H):
            rows = slice(h * 32, (h + 1) * 32)
            q = q_ref[m, rows, :].reshape(4, 8, L)
            qs = [q[i] for i in range(4)]
            if chain and dep is not None:
                qs[0] = _tie(qs[0], dep, zero)
            logits = []
            for w in range(8):
                k = k_ref[m + 8 - w, rows, :].reshape(4, 8, L)
                s = (qs[0] * k[0] + qs[1] * k[1]) + (qs[2] * k[2] + qs[3] * k[3])
                s = s + pltpu.roll(s, 4, 0)
                s = s + pltpu.roll(s, 2, 0)
                s = s + pltpu.roll(s, 1, 0)
                if w > 0 and not (isinstance(m, int) and m >= w):
                    s = jnp.where(jnp.logical_or(lane_ok, m >= w), s, -1e9)
                logits.append(s)
            mx = logits[0]
            for w in range(1, 8):
                mx = jnp.maximum(mx, logits[w])
            es = [jnp.exp2((l - mx) * scale) for l in logits]
            ssum = es[0]
            for w in range(1, 8):
                ssum = ssum + es[w]
            r = _recip(ssum)
            acc = None
            for w in range(8):
                v = v_ref[m + 8 - w, rows, :].reshape(4, 8, L)
                t = v * es[w][None]
                acc = t if acc is None else acc + t
            o = acc * r[None]
            dep = o[0]
            dst[m, rows, :] = o.reshape(32, L).astype(bf16)

    def cp_wob(c):
        return pltpu.make_async_copy(wob_hbm.at[:, pl.ds(c * L, L)], wobraw.at[c], sems.at[64 + c])

    def scope1(xraw, waraw, woaraw, wbraw):
        x3 = x_hbm.reshape(L, 16, D)

        def cp_x(hf, c):
            return pltpu.make_async_copy(x3.at[:, pl.ds(8 * hf, 8), pl.ds(c * L, L)],
                                         xraw.at[c, :, pl.ds(8 * hf, 8), :], sems.at[8 * hf + c])

        def cp_wa(c):
            return pltpu.make_async_copy(wa_hbm.at[:, pl.ds(c * L, L)], waraw.at[c], sems.at[16 + c])

        def cp_wb(c):
            src = (c + 8) % 24
            return pltpu.make_async_copy(wb_hbm.at[:, pl.ds(src * L, L)], wbraw.at[c], sems.at[40 + c])

        def cp_woa(c):
            return pltpu.make_async_copy(woa_hbm.at[:, pl.ds(c * L, L)], woaraw.at[c], sems.at[72 + c])

        for c in range(8):
            cp_x(0, c).start()
        for c in range(3):
            cp_wa(c).start()

        ones = jnp.ones((16, L), bf16)
        for j in range(T):
            for p in range(NP):
                vA[j, 80 * p + 64:80 * p + 80, :] = ones

        rr = lax.broadcasted_iota(i32, (L, L), 0)
        cc = lax.broadcasted_iota(i32, (L, L), 1)
        h_out = (rr // 64) * 2 + (rr % 2)
        keep = h_out == (cc // 32)
        re = lax.broadcasted_iota(i32, (L, DH), 0)
        ce = lax.broadcasted_iota(i32, (L, DH), 1)
        f_out = ((re % 64) // 8) * 4 + (re % 8) // 2
        E = jnp.where(f_out == ce, 1.0, 0.0).astype(bf16)
        G = []
        for c in range(8):
            g = lax.dot_general(E, wphi_ref[c * L:(c + 1) * L, :], NT_DIMS, preferred_element_type=f32)
            G.append(jnp.where(keep, g, 0.0).astype(bf16))

        xv = xraw.bitcast(i32)

        def xin(t):
            for c in range(8):
                wt = xv[c, :, t, :].T
                xT[t, c * L:(c + 1) * L, :] = pltpu.bitcast(wt << 16, f32)
                xT[8 + t, c * L:(c + 1) * L, :] = pltpu.bitcast(wt & jnp.int32(-65536), f32)

        for c in range(8):
            cp_x(0, c).wait()
        for c in range(3, 8):
            cp_wa(c).start()
        xin(0)
        ln(0, xnE)
        ln(8, xnO)

        def wblk(c):
            if c < 16:
                wt = lax.dot_general(G[c % 8], waraw[c], NT_DIMS, preferred_element_type=f32).astype(bf16)
            else:
                wt = waraw[c].T
            waT[64 * c:64 * c + 64, :] = _pk(wt)
            return wt

        def blk_dot(c, wt):
            rhs = jnp.concatenate([xnE[...], xnO[...]], axis=1)
            r = jnp.dot(wt, rhs, preferred_element_type=f32)
            for u, (j, pqk) in enumerate(((0, pqkE), (8, pqkO))):
                ru = r[:, L * u:L * (u + 1)]
                if c < 16:
                    pqk[L * c:L * (c + 1), :] = ru
                else:
                    v = ru.astype(bf16)
                    for pp in range(2):
                        p = 2 * (c - 16) + pp
                        vA[j, 80 * p:80 * p + 64, :] = v[64 * pp:64 * pp + 64]

        def blocks(c0, c1):
            for c in range(c0, c1):
                cp_wa(c).wait()
                if c + 8 < 24:
                    cp_wa(c + 8).start()
            wts = [wblk(c) for c in range(c0, c1)]
            for c in range(c0, c1):
                blk_dot(c, wts[c - c0])

        blocks(0, 2)
        blocks(2, 5)
        blocks(5, 8)

        def mid(c0, c1, extra):
            blocks(c0, c1)
            extra()
        for c in range(8):
            cp_x(1, c).start()
        region(mid, 8, 16, lambda: (xin(1), ln(1, xn_tmp(1)), ln(9, xn_tmp(9)), xin(2), xin(3)))
        for c in range(24):
            cp_wb(c).start()
        for c in range(8):
            cp_woa(c).start()
        for c in range(8):
            cp_wob(c).start()
        region(blocks, 16, 24)

        def wait_wb(c):
            pltpu.make_async_copy(wb_hbm.at[:, pl.ds(0, L)], wbraw.at[c], sems.at[40 + c]).wait()

        def xpose_wb(c):
            wbT[pl.ds(pl.multiple_of(64 * c, 64), 64), :] = _pk(wbraw[c].T)

        def body(t, carry, src=None, extra=None):
            for u in range(4):
                wait_wb(4 * (t - 1) + u)
            soft_a(t - 1, pqkE)
            soft_a(t + 7, pqkO)
            qkv_a(t, xnE if src is None else src[0], pqkE)
            qkv_a(t + 8, xnO if src is None else src[1], pqkO)
            if extra is not None:
                extra()
            ln(t + 1, xnE)
            ln(t + 9, xnO)
            for u in range(4):
                xpose_wb(4 * (t - 1) + u)
            return carry

        for c in range(8):
            cp_x(1, c).wait()
        region(body, 1, 0, (xn.at[1], xn.at[9]), lambda: [xin(t) for t in range(4, 8)])
        lax.fori_loop(2, 7, body, 0)
        for c in range(8):
            cp_woa(c).wait()
        soft_a(6, pqkE)
        soft_a(14, pqkO)
        qkv_a(7, xnE, pqkE)
        qkv_a(15, xnO, pqkO)
        for c in range(8):
            woaT[64 * c:64 * c + 64, :] = _pk(woaraw[c].T)
        soft_a(7, pqkE)
        soft_a(15, pqkO)
        kv_phase()

    pl.run_scoped(scope1,
                  pltpu.VMEM((8, L, 16, L), bf16), pltpu.VMEM((24, D, L), bf16), pltpu.VMEM((8, D, L), bf16),
                  pltpu.VMEM((24, D, L), bf16))

    def scope2(qE, kE, vE, qO, kO, vO, ostage):
        def attn_e(m, chain=True):
            attn_b(oS, m, qE, kE, vE, chain)

        def attn_o(m, chain=True):
            attn_b(oB, m, qO, kO, vO, chain)

        def b1(first):
            num_phase()
            oproj(0, woaT)
            oproj(1, woaT)
            ln_arr(0)

            def step(i, odd, do_o=True, do_ln=True, wob=False):
                if do_o:
                    oproj(i + 2, woaT)
                if odd:
                    attn_e(i - 8)
                    qkv_b(i, i - 8, qO, kO, vO)
                else:
                    qkv_b(i, i, qE, kE, vE)
                if do_ln:
                    ln_arr(i + 1)
                if wob:
                    wobT[pl.ds(pl.multiple_of(64 * i, 64), 64), :] = _pk(wobraw[i].T)

            def bodyx(i, carry):
                if first:
                    cp_wob(i).wait()
                step(i, False, wob=first)
                return carry
            lax.fori_loop(0, 8, bodyx, 0)

            def bodyy(i, carry):
                step(i, True)
                return carry
            lax.fori_loop(8, 14, bodyy, 0)
            region(step, 14, True, False)
            region(step, 15, True, False, False)

        b1(True)
        def z0():
            oproj(0, wobT)
            attn_o(0, False)
            oproj(1, wobT)

        def z1():
            oproj(8, wobT, True)
            attn_o(1)
            ln(0, xnE)

        def z2():
            oproj(9, wobT, True)
            attn_o(2)
            ln(8, xnO)

        region(z0)
        region(z1)
        region(z2)

        def bodyz(t, carry):
            oproj(t + 1, wobT)
            oproj(t + 9, wobT, True)
            soft_a(jnp.maximum(t - 2, 0), pqkE)
            soft_a(jnp.maximum(t - 2, 0) + 8, pqkO)
            qkv_a(t - 1, xnE, pqkE)
            qkv_a(t + 7, xnO, pqkO)
            ln(t, xnE)
            ln(t + 8, xnO)
            attn_o(jnp.minimum(t + 2, 7))
            return carry
        lax.fori_loop(1, 7, bodyz, 0)
        soft_a(5, pqkE)
        soft_a(13, pqkO)
        qkv_a(6, xnE, pqkE)
        qkv_a(14, xnO, pqkO)
        ln(7, xnE)
        ln(15, xnO)
        soft_a(6, pqkE)
        soft_a(14, pqkO)
        qkv_a(7, xnE, pqkE)
        qkv_a(15, xnO, pqkO)
        soft_a(7, pqkE)
        soft_a(15, pqkO)
        kv_phase()

        b1(False)
        ov = ostage.bitcast(i32)

        def oproj_c(c, par):
            rhs = jnp.concatenate([(oB if par else oS)[m] for m in range(8)], axis=1)
            y = jnp.dot(_bf(wobT[pl.ds(pl.multiple_of(64 * c, 64), 64), :]), rhs, preferred_element_type=f32)
            rows = pl.ds(pl.multiple_of(c * L, L), L)
            for m in range(8):
                j = 8 * par + m
                xT[j, rows, :] = xT[j, rows, :] + y[:, L * m:L * (m + 1)]

        def pack_c(c):
            rows = pl.ds(pl.multiple_of(c * L, L), L)
            for t in range(8):
                wv = pltpu.pack_elementwise([xT[t, rows, :], xT[t + 8, rows, :]], packed_dtype=bf16)
                ov[c, pl.ds(t, L, stride=8), :] = pltpu.bitcast(wv, i32).T

        def out_cp(c):
            return pltpu.make_async_copy(ostage.at[c], out_hbm.at[:, pl.ds(c * L, L)], sems.at[c])

        def f1(c, carry):
            attn_o(c)
            oproj_c(c, 0)
            return carry
        lax.fori_loop(0, 8, f1, 0)

        def f2(c, carry):
            pack_c(c - 1)
            out_cp(c - 1).start()
            oproj_c(c, 1)
            return carry
        region(oproj_c, 0, 1)
        lax.fori_loop(1, 8, f2, 0)
        pack_c(7)
        out_cp(7).start()
        for c in range(8):
            out_cp(c).wait()

    pl.run_scoped(scope2,
                  pltpu.VMEM((8, D, L), f32), pltpu.VMEM((16, D, L), f32), pltpu.VMEM((16, D, L), f32),
                  pltpu.VMEM((8, D, L), f32), pltpu.VMEM((16, D, L), f32), pltpu.VMEM((16, D, L), f32),
                  pltpu.VMEM((8, S, L), bf16))


@jax.jit
def pallas_interleave_layers__linear_kernel_hedgehog__sliding_local_dilated__prompt_kernel(
        A_x, A_wqkv, A_w_phi, A_wo, B_x, B_wqkv, B_wo):
    del B_x
    x = A_x.reshape(S, D)
    wphi = A_w_phi.reshape(H * DH, DH)
    any_spec = pl.BlockSpec(memory_space=pl.ANY)
    out = pl.pallas_call(
        _kernel,
        out_shape=jax.ShapeDtypeStruct((S, D), bf16),
        in_specs=[pl.BlockSpec(memory_space=pltpu.SMEM), any_spec, any_spec, pl.BlockSpec(memory_space=pltpu.VMEM), any_spec, any_spec, any_spec],
        out_specs=any_spec,
        scratch_shapes=[
            pltpu.VMEM((1536, D), i32),
            pltpu.VMEM((1536, D), i32),
            pltpu.VMEM((512, D), i32),
            pltpu.VMEM((512, D), i32),
            pltpu.VMEM((8, D, L), bf16),
            pltpu.VMEM((T, D, L), f32),
            pltpu.VMEM((T, D, L), bf16),
            pltpu.VMEM((D, L), bf16),
            pltpu.VMEM((D, L), bf16),
            pltpu.VMEM((2048, L), f32),
            pltpu.VMEM((2048, L), f32),
            pltpu.VMEM((T, 2048, L), bf16),
            pltpu.VMEM((T, 2048, L), bf16),
            pltpu.VMEM((T, 1280, L), bf16),
            pltpu.VMEM((T, D, L), bf16),
            pltpu.VMEM((8, D, L), bf16),
            pltpu.VMEM((NP, 80, L), bf16),
            pltpu.SemaphoreType.DMA((80,)),
        ],
        compiler_params=pltpu.CompilerParams(vmem_limit_bytes=120 * 1024 * 1024),
        name="hedgehog_fused",
    )(np.ones((1,), np.int32), x, A_wqkv, wphi, A_wo, B_wqkv, B_wo)
    return out.reshape(1, S, D)
```

```python
import jax
import jax.numpy as jnp
import numpy as np
from jax import lax
from jax.experimental import pallas as pl
from jax.experimental.pallas import tpu as pltpu

bf16 = jnp.bfloat16
f32 = jnp.float32
i32 = jnp.int32

S, D, H, DH = 2048, 1024, 32, 32
T, L = 16, 128
NP = 16
LOG2E = 1.4426950408889634
NT_DIMS = (((1,), (1,)), ((), ()))


def _bf(x):
    return pltpu.bitcast(x, bf16)


def _pk(x):
    return pltpu.bitcast(x, i32)


def _recip(x):
    r = pltpu.reciprocal(x, approx=True)
    return r * (2.0 - x * r)


def _layernorm(xT, j, store):
    CH = 64
    n = D // CH
    acc = [None] * 4
    for c in range(n):
        s = jnp.sum(xT[j, c * CH:(c + 1) * CH, :].reshape(CH // 8, 8, L), axis=0)
        acc[c % 4] = s if acc[c % 4] is None else acc[c % 4] + s
    m = jnp.sum((acc[0] + acc[1]) + (acc[2] + acc[3]), axis=0, keepdims=True) * (1.0 / D)
    mb = jnp.broadcast_to(m, (8, L))
    acc = [None] * 4
    CH2 = CH // 2
    for c in range(2 * n):
        x = xT[j, c * CH2:(c + 1) * CH2, :].reshape(CH2 // 8, 8, L) - mb[None]
        s = jnp.sum(x * x, axis=0)
        acc[c % 4] = s if acc[c % 4] is None else acc[c % 4] + s
    v = jnp.sum((acc[0] + acc[1]) + (acc[2] + acc[3]), axis=0, keepdims=True) * (1.0 / D)
    r = jnp.broadcast_to(lax.rsqrt(v + 1e-5), (8, L))
    CH3 = CH // 4
    for c in range(4 * n):
        x = (xT[j, c * CH3:(c + 1) * CH3, :].reshape(CH3 // 8, 8, L) - mb[None]) * r[None]
        store(c * CH3, CH3, x.reshape(CH3, L).astype(bf16))


def _dual_softmax_pair(p):
    p3 = p.reshape(8, 8, L) * LOG2E
    mx = jnp.max(p3, axis=0)
    mx = jnp.maximum(mx, pltpu.roll(mx, 4, 0))
    mx = jnp.maximum(mx, pltpu.roll(mx, 2, 0))
    mn = jnp.min(p3, axis=0)
    mn = jnp.minimum(mn, pltpu.roll(mn, 4, 0))
    mn = jnp.minimum(mn, pltpu.roll(mn, 2, 0))
    ep = jnp.exp2(p3 - mx[None])
    en = jnp.exp2(mn[None] - p3)
    sp = jnp.sum(ep, axis=0)
    sp = sp + pltpu.roll(sp, 4, 0)
    sp = sp + pltpu.roll(sp, 2, 0)
    sn = jnp.sum(en, axis=0)
    sn = sn + pltpu.roll(sn, 4, 0)
    sn = sn + pltpu.roll(sn, 2, 0)
    ep = ep * _recip(sp)[None]
    en = en * _recip(sn)[None]
    return jnp.concatenate([ep.reshape(64, L), en.reshape(64, L)], axis=0).astype(bf16)


def _tie(x, dep, zero):
    return pltpu.bitcast(pltpu.bitcast(x, i32) | (pltpu.bitcast(dep, i32) & zero), f32)


def _kernel(one_ref, x_hbm, wa_hbm, wphi_ref, woa_hbm, wb_hbm, wob_hbm, out_hbm,
            waT, wbT, woaT, wobT, wobraw, xT, xn, xnE, xnO, pqkE, pqkO, phiq, phik, vA, oS, oB, numL, sems):
    def region(fn, *args):
        def run():
            fn(*args)
        pl.when(one_ref[0] > 0)(run)

    zero = lax.broadcasted_iota(i32, (8, L), 1) >> 10
    lane_ok = lax.broadcasted_iota(i32, (8, L), 1) >= 1

    def ln(j, dst):
        def store(r0, n, val):
            dst[r0:r0 + n, :] = val
        _layernorm(xT, j, store)

    def xn_tmp(j):
        return xn.at[j]

    def ln_arr(j):
        def store(r0, n, val):
            xn[j, r0:r0 + n, :] = val
        _layernorm(xT, j, store)

    def qkv_a(j, src, pqk):
        r = jnp.dot(_bf(waT[...]), src[...], preferred_element_type=f32)
        pqk[...] = r[0:2048]
        v = r[2048:3072].astype(bf16)
        for p in range(NP):
            vA[j, 80 * p:80 * p + 64, :] = v[64 * p:64 * p + 64]

    def soft_a(j, pqk):
        for p in range(NP):
            phiq[j, 128 * p:128 * p + 128, :] = _dual_softmax_pair(pqk[64 * p:64 * p + 64, :])
            phik[j, 128 * p:128 * p + 128, :] = _dual_softmax_pair(pqk[1024 + 64 * p:1024 + 64 * p + 64, :])

    def kv_phase():
        r = lax.broadcasted_iota(i32, (80, L), 0)
        c = lax.broadcasted_iota(i32, (80, L), 1)
        hs = jnp.where(r < 64, r // 32, (r - 64) // 8)
        keep = hs == (c % 2)
        for p in range(NP):
            Lm = jnp.concatenate([vA[j, 80 * p:80 * p + 80, :] for j in range(T)], axis=1)
            Rm = jnp.concatenate([phik[j, 128 * p:128 * p + 128, :] for j in range(T)], axis=1)
            kvT = lax.dot_general(Lm, Rm, NT_DIMS, preferred_element_type=f32)
            numL[p] = jnp.where(keep, kvT, 0.0).astype(bf16)

    def num_phase():
        for p in range(NP):
            Rm = jnp.concatenate([phiq[j, 128 * p:128 * p + 128, :] for j in range(T)], axis=1)
            nd = jnp.dot(numL[p], Rm, preferred_element_type=f32)
            for j in range(T):
                t = nd[:, L * j:L * (j + 1)]
                r0 = _recip(t[64:72] + 1e-6)
                r1 = _recip(t[72:80] + 1e-6)
                o0 = (t[0:32].reshape(4, 8, L) * r0[None]).reshape(32, L)
                o1 = (t[32:64].reshape(4, 8, L) * r1[None]).reshape(32, L)
                oS[j, 64 * p:64 * p + 64, :] = jnp.concatenate([o0, o1], axis=0).astype(bf16)

    def oproj(j, woT, odd_b=False):
        src = oB[j - 8] if odd_b else oS[j]
        y = jnp.dot(_bf(woT[...]), src, preferred_element_type=f32)
        xT[j] = xT[j] + y

    def qkv_b(j, m, q_ref, k_ref, v_ref):
        r = jnp.dot(_bf(wbT[...]), xn[j], preferred_element_type=f32)
        CH = 64
        for ref, off in ((k_ref, 0), (v_ref, 1024)):
            for c in range(D // CH):
                val = r[off + c * CH:off + (c + 1) * CH]
                ref[m + 8, c * CH:(c + 1) * CH, :] = val
                ref[m, c * CH:(c + 1) * CH, :] = pltpu.roll(val, 1, 1)
        q_ref[m] = r[2048:3072]

    def attn_b(dst, m, q_ref, k_ref, v_ref, chain):
        scale = DH ** -0.5 * LOG2E
        dep = None
        for h in range(H):
            rows = slice(h * 32, (h + 1) * 32)
            q = q_ref[m, rows, :].reshape(4, 8, L)
            qs = [q[i] for i in range(4)]
            if chain and dep is not None:
                qs[0] = _tie(qs[0], dep, zero)
            logits = []
            for w in range(8):
                k = k_ref[m + 8 - w, rows, :].reshape(4, 8, L)
                s = (qs[0] * k[0] + qs[1] * k[1]) + (qs[2] * k[2] + qs[3] * k[3])
                s = s + pltpu.roll(s, 4, 0)
                s = s + pltpu.roll(s, 2, 0)
                s = s + pltpu.roll(s, 1, 0)
                if w > 0 and not (isinstance(m, int) and m >= w):
                    s = jnp.where(jnp.logical_or(lane_ok, m >= w), s, -1e9)
                logits.append(s)
            mx = logits[0]
            for w in range(1, 8):
                mx = jnp.maximum(mx, logits[w])
            es = [jnp.exp2((l - mx) * scale) for l in logits]
            ssum = es[0]
            for w in range(1, 8):
                ssum = ssum + es[w]
            r = _recip(ssum)
            acc = None
            for w in range(8):
                v = v_ref[m + 8 - w, rows, :].reshape(4, 8, L)
                t = v * es[w][None]
                acc = t if acc is None else acc + t
            o = acc * r[None]
            dep = o[0]
            dst[m, rows, :] = o.reshape(32, L).astype(bf16)

    def cp_wob(c):
        return pltpu.make_async_copy(wob_hbm.at[:, pl.ds(c * L, L)], wobraw.at[c], sems.at[64 + c])

    def scope1(xraw, waraw, woaraw, wbraw):
        x3 = x_hbm.reshape(L, 16, D)

        def cp_x(hf, c):
            return pltpu.make_async_copy(x3.at[:, pl.ds(8 * hf, 8), pl.ds(c * L, L)],
                                         xraw.at[c, :, pl.ds(8 * hf, 8), :], sems.at[8 * hf + c])

        def cp_wa(c):
            return pltpu.make_async_copy(wa_hbm.at[:, pl.ds(c * L, L)], waraw.at[c], sems.at[16 + c])

        def cp_wb(c):
            src = (c + 8) % 24
            return pltpu.make_async_copy(wb_hbm.at[:, pl.ds(src * L, L)], wbraw.at[c], sems.at[40 + c])

        def cp_woa(c):
            return pltpu.make_async_copy(woa_hbm.at[:, pl.ds(c * L, L)], woaraw.at[c], sems.at[72 + c])

        for c in range(8):
            cp_x(0, c).start()
        for c in range(3):
            cp_wa(c).start()

        ones = jnp.ones((16, L), bf16)
        for j in range(T):
            for p in range(NP):
                vA[j, 80 * p + 64:80 * p + 80, :] = ones

        rr = lax.broadcasted_iota(i32, (L, L), 0)
        cc = lax.broadcasted_iota(i32, (L, L), 1)
        h_out = (rr // 64) * 2 + (rr % 2)
        keep = h_out == (cc // 32)
        re = lax.broadcasted_iota(i32, (L, DH), 0)
        ce = lax.broadcasted_iota(i32, (L, DH), 1)
        f_out = ((re % 64) // 8) * 4 + (re % 8) // 2
        E = jnp.where(f_out == ce, 1.0, 0.0).astype(bf16)
        G = []
        for c in range(8):
            g = lax.dot_general(E, wphi_ref[c * L:(c + 1) * L, :], NT_DIMS, preferred_element_type=f32)
            G.append(jnp.where(keep, g, 0.0).astype(bf16))

        xv = xraw.bitcast(i32)

        def xin(t):
            for c in range(8):
                wt = xv[c, :, t, :].T
                xT[t, c * L:(c + 1) * L, :] = pltpu.bitcast(wt << 16, f32)
                xT[8 + t, c * L:(c + 1) * L, :] = pltpu.bitcast(wt & jnp.int32(-65536), f32)

        for c in range(8):
            cp_x(0, c).wait()
        for c in range(3, 8):
            cp_wa(c).start()
        xin(0)
        ln(0, xnE)
        ln(8, xnO)

        def wblk(c):
            if c < 16:
                wt = lax.dot_general(G[c % 8], waraw[c], NT_DIMS, preferred_element_type=f32).astype(bf16)
            else:
                wt = waraw[c].T
            waT[64 * c:64 * c + 64, :] = _pk(wt)
            return wt

        def blk_dot(c, wt):
            rhs = jnp.concatenate([xnE[...], xnO[...]], axis=1)
            r = jnp.dot(wt, rhs, preferred_element_type=f32)
            for u, (j, pqk) in enumerate(((0, pqkE), (8, pqkO))):
                ru = r[:, L * u:L * (u + 1)]
                if c < 16:
                    pqk[L * c:L * (c + 1), :] = ru
                else:
                    v = ru.astype(bf16)
                    for pp in range(2):
                        p = 2 * (c - 16) + pp
                        vA[j, 80 * p:80 * p + 64, :] = v[64 * pp:64 * pp + 64]

        def blocks(c0, c1):
            for c in range(c0, c1):
                cp_wa(c).wait()
                if c + 8 < 24:
                    cp_wa(c + 8).start()
            wts = [wblk(c) for c in range(c0, c1)]
            for c in range(c0, c1):
                blk_dot(c, wts[c - c0])

        blocks(0, 2)
        blocks(2, 5)
        blocks(5, 8)

        def mid(c0, c1, extra):
            blocks(c0, c1)
            extra()
        for c in range(8):
            cp_x(1, c).start()
        region(mid, 8, 16, lambda: (xin(1), ln(1, xn_tmp(1)), ln(9, xn_tmp(9)), xin(2), xin(3)))
        for c in range(24):
            cp_wb(c).start()
        for c in range(8):
            cp_woa(c).start()
        for c in range(8):
            cp_wob(c).start()
        region(blocks, 16, 24)

        def wait_wb(c):
            pltpu.make_async_copy(wb_hbm.at[:, pl.ds(0, L)], wbraw.at[c], sems.at[40 + c]).wait()

        def xpose_wb(c):
            wbT[pl.ds(pl.multiple_of(64 * c, 64), 64), :] = _pk(wbraw[c].T)

        def body(t, carry, src=None, extra=None):
            for u in range(4):
                wait_wb(4 * (t - 1) + u)
            soft_a(t - 1, pqkE)
            soft_a(t + 7, pqkO)
            qkv_a(t, xnE if src is None else src[0], pqkE)
            qkv_a(t + 8, xnO if src is None else src[1], pqkO)
            if extra is not None:
                extra()
            ln(t + 1, xnE)
            ln(t + 9, xnO)
            for u in range(4):
                xpose_wb(4 * (t - 1) + u)
            return carry

        for c in range(8):
            cp_x(1, c).wait()
        region(body, 1, 0, (xn.at[1], xn.at[9]), lambda: [xin(t) for t in range(4, 6)])
        region(body, 2, 0, None, lambda: [xin(t) for t in range(6, 8)])
        lax.fori_loop(3, 7, body, 0)
        for c in range(8):
            cp_woa(c).wait()
        soft_a(6, pqkE)
        soft_a(14, pqkO)
        qkv_a(7, xnE, pqkE)
        qkv_a(15, xnO, pqkO)
        for c in range(8):
            woaT[64 * c:64 * c + 64, :] = _pk(woaraw[c].T)
        soft_a(7, pqkE)
        soft_a(15, pqkO)
        kv_phase()

    pl.run_scoped(scope1,
                  pltpu.VMEM((8, L, 16, L), bf16), pltpu.VMEM((24, D, L), bf16), pltpu.VMEM((8, D, L), bf16),
                  pltpu.VMEM((24, D, L), bf16))

    def scope2(qE, kE, vE, qO, kO, vO, ostage):
        def attn_e(m, chain=True):
            attn_b(oS, m, qE, kE, vE, chain)

        def attn_o(m, chain=True):
            attn_b(oB, m, qO, kO, vO, chain)

        def b1(first):
            num_phase()
            oproj(0, woaT)
            oproj(1, woaT)
            ln_arr(0)

            def step(i, odd, do_o=True, do_ln=True, wob=False):
                if do_o:
                    oproj(i + 2, woaT)
                if odd:
                    attn_e(i - 8)
                    qkv_b(i, i - 8, qO, kO, vO)
                else:
                    qkv_b(i, i, qE, kE, vE)
                if do_ln:
                    ln_arr(i + 1)
                if wob:
                    wobT[pl.ds(pl.multiple_of(64 * i, 64), 64), :] = _pk(wobraw[i].T)

            def bodyx(i, carry):
                if first:
                    cp_wob(i).wait()
                step(i, False, wob=first)
                return carry
            lax.fori_loop(0, 8, bodyx, 0)

            def bodyy(i, carry):
                step(i, True)
                return carry
            lax.fori_loop(8, 14, bodyy, 0)
            region(step, 14, True, False)
            region(step, 15, True, False, False)

        b1(True)
        def z0():
            oproj(0, wobT)
            attn_o(0, False)
            oproj(1, wobT)

        def z1():
            oproj(8, wobT, True)
            attn_o(1)
            ln(0, xnE)

        def z2():
            oproj(9, wobT, True)
            attn_o(2)
            ln(8, xnO)

        region(z0)
        region(z1)
        region(z2)

        def bodyz(t, carry):
            oproj(t + 1, wobT)
            oproj(t + 9, wobT, True)
            soft_a(jnp.maximum(t - 2, 0), pqkE)
            soft_a(jnp.maximum(t - 2, 0) + 8, pqkO)
            qkv_a(t - 1, xnE, pqkE)
            qkv_a(t + 7, xnO, pqkO)
            ln(t, xnE)
            ln(t + 8, xnO)
            attn_o(jnp.minimum(t + 2, 7))
            return carry
        lax.fori_loop(1, 7, bodyz, 0)
        soft_a(5, pqkE)
        soft_a(13, pqkO)
        qkv_a(6, xnE, pqkE)
        qkv_a(14, xnO, pqkO)
        ln(7, xnE)
        ln(15, xnO)
        soft_a(6, pqkE)
        soft_a(14, pqkO)
        qkv_a(7, xnE, pqkE)
        qkv_a(15, xnO, pqkO)
        soft_a(7, pqkE)
        soft_a(15, pqkO)
        kv_phase()

        b1(False)
        ov = ostage.bitcast(i32)

        def oproj_c(c, par):
            rhs = jnp.concatenate([(oB if par else oS)[m] for m in range(8)], axis=1)
            y = jnp.dot(_bf(wobT[64 * c:64 * c + 64, :]), rhs, preferred_element_type=f32)
            rows = slice(c * L, (c + 1) * L)
            for m in range(8):
                j = 8 * par + m
                xT[j, rows, :] = xT[j, rows, :] + y[:, L * m:L * (m + 1)]

        def pack_c(c):
            rows = slice(c * L, (c + 1) * L)
            for t in range(8):
                wv = pltpu.pack_elementwise([xT[t, rows, :], xT[t + 8, rows, :]], packed_dtype=bf16)
                ov[c, pl.ds(t, L, stride=8), :] = pltpu.bitcast(wv, i32).T

        def out_cp(c):
            return pltpu.make_async_copy(ostage.at[c], out_hbm.at[:, pl.ds(c * L, L)], sems.at[c])

        def f1(c):
            attn_o(c)
            oproj_c(c, 0)

        def f2(c):
            oproj_c(c, 1)
            if c >= 1:
                pack_c(c - 1)

        for c in range(8):
            region(f1, c)
        for c in range(8):
            region(f2, c)
            if c >= 1:
                out_cp(c - 1).start()
        pack_c(7)
        out_cp(7).start()
        for c in range(8):
            out_cp(c).wait()

    pl.run_scoped(scope2,
                  pltpu.VMEM((8, D, L), f32), pltpu.VMEM((16, D, L), f32), pltpu.VMEM((16, D, L), f32),
                  pltpu.VMEM((8, D, L), f32), pltpu.VMEM((16, D, L), f32), pltpu.VMEM((16, D, L), f32),
                  pltpu.VMEM((8, S, L), bf16))


@jax.jit
def pallas_interleave_layers__linear_kernel_hedgehog__sliding_local_dilated__prompt_kernel(
        A_x, A_wqkv, A_w_phi, A_wo, B_x, B_wqkv, B_wo):
    del B_x
    x = A_x.reshape(S, D)
    wphi = A_w_phi.reshape(H * DH, DH)
    any_spec = pl.BlockSpec(memory_space=pl.ANY)
    out = pl.pallas_call(
        _kernel,
        out_shape=jax.ShapeDtypeStruct((S, D), bf16),
        in_specs=[pl.BlockSpec(memory_space=pltpu.SMEM), any_spec, any_spec, pl.BlockSpec(memory_space=pltpu.VMEM), any_spec, any_spec, any_spec],
        out_specs=any_spec,
        scratch_shapes=[
            pltpu.VMEM((1536, D), i32),
            pltpu.VMEM((1536, D), i32),
            pltpu.VMEM((512, D), i32),
            pltpu.VMEM((512, D), i32),
            pltpu.VMEM((8, D, L), bf16),
            pltpu.VMEM((T, D, L), f32),
            pltpu.VMEM((T, D, L), bf16),
            pltpu.VMEM((D, L), bf16),
            pltpu.VMEM((D, L), bf16),
            pltpu.VMEM((2048, L), f32),
            pltpu.VMEM((2048, L), f32),
            pltpu.VMEM((T, 2048, L), bf16),
            pltpu.VMEM((T, 2048, L), bf16),
            pltpu.VMEM((T, 1280, L), bf16),
            pltpu.VMEM((T, D, L), bf16),
            pltpu.VMEM((8, D, L), bf16),
            pltpu.VMEM((NP, 80, L), bf16),
            pltpu.SemaphoreType.DMA((80,)),
        ],
        compiler_params=pltpu.CompilerParams(vmem_limit_bytes=120 * 1024 * 1024),
        name="hedgehog_fused",
    )(np.ones((1,), np.int32), x, A_wqkv, wphi, A_wo, B_wqkv, B_wo)
    return out.reshape(1, S, D)
```
